```python
import os as _os
_os.environ.setdefault("JAX_PLATFORMS", "cpu")
import jax
import jax.numpy as jnp

def _softmax(x, axis=-1):
    return jax.nn.softmax(x, axis=axis)
def _gelu(x):
    return jax.nn.gelu(x, approximate=True)
def _silu(x):
    return jax.nn.silu(x)
def _sigmoid(x):
    return jax.nn.sigmoid(x)
def _layernorm(x, axis=-1, eps=1e-5):
    m = jnp.mean(x, axis=axis, keepdims=True)
    v = jnp.var(x, axis=axis, keepdims=True)
    return (x - m) / jnp.sqrt(v + eps)
def _scatter_add(tgt, idx, src, axis=0):
    return tgt.at[idx].add(src)
def _segment_sum(src, seg, n):
    return jax.ops.segment_sum(src, seg, n)
class _Rng:
    def __init__(self, key):
        self._k = key
    def _next(self):
        self._k, sub = jax.random.split(self._k)
        return sub
    def normal(self, shape):
        return jax.random.normal(self._next(), shape, dtype=jnp.bfloat16)
    def randint(self, lo, hi, shape):
        return jax.random.randint(self._next(), shape, lo, hi, dtype=jnp.int32)
    def uniform(self, shape, lo=0.0, hi=1.0):
        return jax.random.uniform(self._next(), shape, jnp.bfloat16, lo, hi)
    def permutation(self, n):
        return jax.random.permutation(self._next(), n)


kernel_name = 'interleave_layers__linear_attn_block__mha_block__prompt'

def setup_inputs():
    _rng = _Rng(jax.random.key(int.from_bytes(__import__("os").urandom(4), "little")))
    _w = (lambda a: (lambda t: t.astype(jnp.bfloat16) if jnp.issubdtype(t.dtype, jnp.floating) else t)(jnp.asarray(a)))
    def _A_setup():
        B, S, D = 1, 2048, 1024
        return {
            "x": _w((lambda *s: _rng.normal(s) * 0.05)(B, S, D)),
            "wqkv": _w((lambda *s: _rng.normal(s) * 0.1)(D, 3 * D)),
            "wo": _w((lambda *s: _rng.normal(s) * 0.1)(D, D)),
        }
    _A_in = _A_setup()

    def _B_setup():
        B, S, D, H = 1, 2048, 1024, 32
        return {
            "x": _w((lambda *s: _rng.normal(s) * 0.05)(B, S, D)),
            "wqkv": _w((lambda *s: _rng.normal(s) * 0.1)(D, 3 * D)),
            "wo": _w((lambda *s: _rng.normal(s) * 0.05)(D, D)),
        }
    _B_in = _B_setup()

    return {
        "A_x": _A_in["x"],
        "A_wqkv": _A_in["wqkv"],
        "A_wo": _A_in["wo"],
        "B_x": _B_in["x"],
        "B_wqkv": _B_in["wqkv"],
        "B_wo": _B_in["wo"],
    }

def reference(A_x, A_wqkv, A_wo, B_x, B_wqkv, B_wo):
    def _A_ref(x, wqkv, wo):
        B, S, D = x.shape
        H = 32; Dh = D // H
        qkv = (lambda x, *d: x.transpose(*d))((x @ wqkv).reshape(B, S, 3, H, Dh), 2, 0, 3, 1, 4)
        q, k, v = qkv[0], qkv[1], qkv[2]
        phi = lambda t: jnp.where(t > 0, t + 1, jnp.exp(t)) + 1e-6
        pq, pk = phi(q), phi(k)
        kv = jnp.einsum("bhsd,bhse->bhde", pk, v)
        z = jnp.einsum("bhsd->bhd", pk)
        num = jnp.einsum("bhqd,bhde->bhqe", pq, kv)
        den = jnp.einsum("bhqd,bhd->bhq", pq, z)[..., None] + 1e-6
        o = num / den
        return (lambda x, *d: x.transpose(*d))(o, 0, 2, 1, 3).reshape(B, S, D) @ wo

    def _B_ref(x, wqkv, wo):
        B, S, D = x.shape
        H = 32
        Dh = D // H
        qkv = (lambda x, *d: x.transpose(*d))((x @ wqkv).reshape(B, S, 3, H, Dh), 2, 0, 3, 1, 4)
        q, k, v = qkv[0], qkv[1], qkv[2]
        scores = jnp.einsum("bhqd,bhkd->bhqk", q, k) * (Dh ** -0.5)
        p = _softmax(scores, axis=-1)
        o = jnp.einsum("bhqk,bhkd->bhqd", p, v)
        return (lambda x, *d: x.transpose(*d))(o, 0, 2, 1, 3).reshape(B, S, D) @ wo

    x = A_x
    x = x + _A_ref(_layernorm(x, axis=-1), A_wqkv, A_wo)
    x = x + _B_ref(_layernorm(x, axis=-1), B_wqkv, B_wo)
    x = x + _A_ref(_layernorm(x, axis=-1), A_wqkv, A_wo)
    x = x + _B_ref(_layernorm(x, axis=-1), B_wqkv, B_wo)
    return x
```

```python
import math

import jax
import jax.numpy as jnp
from jax import lax
import jax.experimental.pallas as pl
import jax.experimental.pallas.tpu as pltpu

S, D, H, DH = 2048, 1024, 32, 32
TC = 512
NC = S // TC
NG = D // 128
KC = 128
VPU_STEPS = (0, 5, 10)
NB, NP = 4, 49
DB, TB = D // NB, TC // NB
F32, BF16, I32 = jnp.float32, jnp.bfloat16, jnp.int32
QSCALE = DH ** -0.5 * math.log2(math.e)

_TN = (((0,), (0,)), ((), ()))
_NT = (((1,), (1,)), ((), ()))


def _tree(op, xs):
    xs = list(xs)
    while len(xs) > 1:
        xs = [op(xs[i], xs[i + 1]) if i + 1 < len(xs) else xs[i]
              for i in range(0, len(xs), 2)]
    return xs[0]


def _rows(x):
    return [x[i:i + 8] for i in range(0, x.shape[0], 8)]


def _cols(x):
    return [x[:, i:i + 128] for i in range(0, x.shape[1], 128)]


def _sublane_sum(x):
    return jnp.broadcast_to(jnp.sum(x, axis=0, keepdims=True), x.shape)


def _bcast_rows(v, n):
    return jnp.concatenate([v] * (n // 8), axis=0)


def _phi(t):
    return jnp.where(t > 0, t + 1.0, jnp.exp(t)) + 1e-6


def _add(a, b):
    return [[x + y for x, y in zip(r, s)] for r, s in zip(a, b)]


def _sub(a, b):
    return [[x - y for x, y in zip(r, s)] for r, s in zip(a, b)]


_LHS = (((1, 0), _add, (1, 1)), ((0, 0), _add, (1, 1)), ((1, 1),), ((0, 0),),
        ((0, 0), _add, (0, 1)), ((1, 0), _sub, (0, 0)), ((0, 1), _sub, (1, 1)))
_RHS = (((0, 0),), ((0, 0), _sub, (1, 1)), ((1, 0), _sub, (0, 0)), ((0, 1), _sub, (1, 1)),
        ((1, 1),), ((0, 0), _sub, (0, 1)), ((1, 0), _sub, (1, 1)))
_DONE = ((1, 0), (0, 1), (1, 1), (0, 0))


def _operand(term, quad):
    return term[1](quad(*term[0]), quad(*term[2])) if len(term) > 1 else quad(*term[0])


def _terms(table, x):
    if len(x) == 1:
        yield x[0][0]
        return
    n = len(x) // 2
    for term in table:
        yield from _terms(table, _operand(
            term, lambda i, j: [r[j * n:(j + 1) * n] for r in x[i * n:(i + 1) * n]]))


def _combine(products, n=NB):
    if n == 1:
        return [[next(products)]]
    m2 = _combine(products, n // 2)
    m1 = _combine(products, n // 2)
    c22 = _sub(m2, m1)
    m4 = _combine(products, n // 2)
    c21, c11 = _add(m2, m4), _add(m1, m4)
    m3 = _combine(products, n // 2)
    c22 = _add(c22, m3)
    m5 = _combine(products, n // 2)
    c12, c11 = _add(m3, m5), _add(c11, m5)
    c22 = _sub(c22, _combine(products, n // 2))
    c11 = _add(c11, _combine(products, n // 2))
    return [r + s for r, s in zip(c11, c12)] + [r + s for r, s in zip(c21, c22)]


def _blk(i, j):
    return slice(i * DB, (i + 1) * DB), slice(j * TB, (j + 1) * TB)


def _rhs_terms(block):
    grid = [[block(*_blk(i, j)) for j in range(NB)] for i in range(NB)]
    return [t.astype(BF16) for t in _terms(_RHS, grid)]


def _each(blocks):
    idx = [(2 * i + a, 2 * j + b) for i, j in _DONE for a, b in _DONE]
    return [(*_blk(i, j), blocks[i][j]) for i, j in idx]


def _run(jobs):
    for job in jobs:
        job()


def _spread(n, parts):
    slots = [[] for _ in range(n)]
    for first, last, jobs in parts:
        for i, job in enumerate(jobs):
            slots[first + i * (last - first) // len(jobs)].append(job)
    return slots


def _after(x, tokens, zero):
    never = jnp.full((8, 128), zero, I32) != 0
    cols = _cols(pltpu.bitcast(x, I32))
    for tok in tokens:
        cols[-1] = jnp.where(never, pltpu.bitcast(tok, I32), cols[-1])
    return pltpu.bitcast(jnp.concatenate(cols, axis=1), BF16)


def _kernel(x_hbm, wa_hbm, woa_hbm, wb_hbm, wob_hbm, out_hbm,
            io_buf, woa, wak, wav, wao, wbv, wbo, wqk, wt,
            xt, stat, act, kvt, zacc, s_buf,
            qt, kk, vt, ks, qr0, qr1, zero_ref, sem_x, sem_w, sem_o):
    waq, wbq, wbk = wqk.at[0], wqk.at[1], wqk.at[2]

    def clear(i, _):
        zero_ref[i] = 0

    lax.fori_loop(0, 2, clear, None)
    uses = iter(range(1, 1000))

    def zero():
        return zero_ref[0] * next(uses)

    def project(w, terms, *side):
        z = zero()
        due = {}

        def products():
            for p, jobs in enumerate(_spread(NP, side)):
                if due.get(p):
                    lhs = jnp.concatenate(
                        [w[p + z, :DB - 16, :], _after(w[p + z, DB - 16:, :], due[p], z)],
                        axis=0)
                else:
                    lhs = w[p + z]
                result = jnp.dot(lhs, terms[p], preferred_element_type=F32)
                due[p + 3] = [tok for job in jobs for tok in job() or ()]
                yield result
        return _combine(products())

    def expand_jobs(w, load, fine):
        z = zero()

        def job(r, qs):
            for q in qs:
                x = _operand(_LHS[q], lambda i, j: [
                    [load(2 * i + a, 2 * j + b, r) for b in range(2)] for a in range(2)])
                for p, t in enumerate(_terms(_LHS, x)):
                    w[7 * q + p, r:r + 8, :] = t.astype(BF16)
            if not fine or r % 16 == 8:
                return [w[7 * qs[-1] + z, r:r + 8, :128].astype(F32)]

        if fine:
            return [lambda r=r, q=q: job(r, [q]) for q in range(7) for r in range(0, DB, 8)]
        return [lambda r=r: job(r, range(7)) for r in range(0, DB, 8)]

    def stats_jobs(c, step=64):
        acc = {}
        z = zero()

        def mean(r):
            t = acc[0] if r else jnp.zeros((8, TC), F32)
            for x in _rows(xt[c + z, r:r + step, :]):
                t = t + x
            acc[0] = _sublane_sum(t) * (1.0 / D) if r + step == D else t
            return _cols(acc[0])

        def variance(r):
            t = acc[1] if r else jnp.zeros((8, TC), F32)
            for x in _rows(xt[c - z, r:r + step, :]):
                t = t + (x - acc[0]) * (x - acc[0])
            acc[1] = t
            if r + step == D:
                stat[0] = acc[0]
                stat[1] = lax.rsqrt(_sublane_sum(t) * (1.0 / D) + 1e-5)
            return _cols(t)

        return [lambda f=f, r=r: f(r) for f in (mean, variance) for r in range(0, D, step)]

    def ln_terms(c):
        mean, rstd = stat[0], stat[1]
        c = c + zero()
        return _rhs_terms(lambda r, t: (
            (xt[c, r, t] - _bcast_rows(mean[:, t], DB)) * _bcast_rows(rstd[:, t], DB)))

    def a_reset():
        kvt[...] = jnp.zeros_like(kvt)
        zacc[...] = jnp.zeros_like(zacc)

    def groups(blocks):
        return [jnp.concatenate([b[r:r + 128] for b in row], axis=1).astype(BF16)
                for row in blocks for r in range(0, DB, 128)]

    def a_k(terms, *side):
        pk = [[_phi(b) for b in row] for row in project(wak, terms, *side)]
        for i, row in enumerate(pk):
            zacc[i * DB:(i + 1) * DB, :] += _tree(jnp.add, row)
        return groups(pk)

    def a_v(terms, *side):
        return groups(project(wav, terms, *side))

    def a_q(c, terms, *side):
        for r, t, b in _each(project(waq, terms, *side)):
            act[c, r, t] = _phi(b)

    def kv_jobs(pk, v):
        def job(g):
            kvt[g] += lax.dot_general(v[g], pk[g], _NT, preferred_element_type=F32)
        return [lambda g=g: job(g) for g in reversed(range(NG))]

    def mix_jobs():
        def job(g):
            r = lax.broadcasted_iota(I32, (128, 128), 0) // DH
            c = lax.broadcasted_iota(I32, (128, 128), 1) // DH
            gs = slice(g * 128, (g + 1) * 128)
            blk = jnp.where(r == c, kvt[g], 0.0).astype(BF16)
            s_buf[g // 2, :D, g % 2 * 128:(g % 2 + 1) * 128] = lax.dot_general(
                woa[gs, :], blk, _TN, preferred_element_type=F32)
            z = jnp.sum(zacc[gs, :], axis=1, keepdims=True)
            zacc[gs, :] = jnp.broadcast_to(z, (128, 128))
        return [lambda g=g: job(g) for g in reversed(range(NG))]

    def a_last_chunk(side_k=(), side_v=()):
        z = zero()
        terms = ln_terms(NC - 1)
        pk = a_k(terms, *side_k)
        v = a_v(terms, *side_v)
        a_q(NC - 1, terms, (1, 2, kv_jobs(pk, v) + mix_jobs()),
            (4, NP - 1, expand_jobs(
                wao, lambda i, j, r: s_buf[j + z, i * DB + r:i * DB + r + 8, :DB], False)))

    def a_out(c):
        c = c + zero()

        def normalised(r, t):
            parts = []
            for h in range(r.start, r.stop, DH):
                p = act[c, h:h + DH, t]
                den = _sublane_sum(_tree(jnp.add, _rows(p * zacc[h:h + DH, :]))) + 1e-6
                parts.append(p * _bcast_rows(1.0 / den, DH))
            return jnp.concatenate(parts, axis=0)

        for r, t, b in _each(project(wao, _rhs_terms(normalised))):
            xt[c, r, t] += b

    def b_chunk(c, last=None):
        def store(ref, blocks, scale=None):
            for i, row in enumerate(blocks):
                for j in range(0, NB, 2):
                    b = jnp.concatenate(row[j:j + 2], axis=1)
                    ref[c, i * DB:(i + 1) * DB, j * TB:(j + 2) * TB] = (
                        b * scale if scale else b).astype(BF16)

        terms = ln_terms(c)
        for r, t, b in _each(project(wbk, terms)):
            for g in range(DB // 128):
                kk[r.start // 128 + g, c, t, :] = b[g * 128:(g + 1) * 128].astype(BF16).T
        if last is None:
            store(qt, project(wbq, terms), QSCALE)
            a_out(c + 1)
            store(vt, project(wbv, terms, (2, NP - 4, stats_jobs(c + 1))))
        else:
            store(qt, project(wbq, terms, *last[:1]), QSCALE)
            store(vt, project(wbv, terms, *last[1:]))

    def b_out(c, *side):
        return _each(project(wbo, _rhs_terms(lambda r, t: act[c, r, t]), *side))

    def skew_keys():
        first = [(n + 1) * KC - 16 for n in VPU_STEPS]
        for g in range(NG):
            x = jnp.concatenate(
                [kk[g, k // TC, k % TC:k % TC + 16, :] for k in first], axis=0).astype(F32)
            row = lax.broadcasted_iota(I32, x.shape, 0)
            lane = lax.broadcasted_iota(I32, x.shape, 1) & (DH - 1)
            for b in (1, 2, 4):
                ahead = jnp.concatenate([x[:, b:], x[:, :b]], axis=1)
                wrapped = jnp.concatenate([x[:, b - DH:], x[:, :b - DH]], axis=1)
                x = jnp.where((row & b) == 0, x, jnp.where(lane < DH - b, ahead, wrapped))
            ks[g] = x

    def head_q(h):
        return qt[h >> 5, pl.ds(pl.multiple_of((h & 31) * DH, DH), DH), :]

    def wrap_q(ref, h):
        for u, q in enumerate(_cols(head_q(h).astype(F32))):
            ref[u] = jnp.concatenate([q, q[:8]], axis=0)

    def attn_jobs(i1, i2, ms, new_ms):
        st = {}
        use_vpu = i1 is not None and i2 is not None
        tiles = [(n, r, u, zero()) for n in range(len(VPU_STEPS))
                 for r in (0, 8) for u in (0, 2)] if use_vpu else []
        vpu = _spread(S // KC, [(3, S // KC, tiles)])

        def fold(name, op, k0, val):
            st[name] = op(st[name], val) if k0 else val

        def vpu_scores(j, n, r, u, z):
            k = ks[(i1 & 7) + z, 16 * n + r:16 * n + r + 8, :]
            for d in range(DH):
                col = jnp.broadcast_to(k[:, j * DH + d:j * DH + d + 1], (8, 128))
                t = [col * (qr0, qr1)[j % 2][u + w, pl.ds(z + d, 8), :] for w in range(2)]
                acc = [x + y for x, y in zip(acc, t)] if d else t
            row = (VPU_STEPS[n] + 1) * KC - 16 + r
            for w in range(2):
                s_buf[j, row:row + 8, (u + w) * 128:(u + w + 1) * 128] = acc[w]
                st["m"][u + w] = jnp.maximum(st["m"][u + w], acc[w])

        def job(j, k0):
            kc, t0 = k0 // TC, k0 % TC
            if i2 is not None:
                s_old = s_buf[j, k0:k0 + KC, :]
            if i1 is not None:
                if k0 == 0:
                    q = head_q(4 * i1 + j)
                    st["q"] = jnp.concatenate(
                        [q if u == j else jnp.zeros_like(q) for u in range(4)], axis=0)
                nk = KC - 16 if use_vpu and k0 // KC in VPU_STEPS else KC
                s = jnp.dot(kk[i1 & 7, kc, t0:t0 + nk, :], st["q"],
                            preferred_element_type=F32)
                s_buf[j, k0:k0 + nk, :] = s
                fold("m", lambda a, b: [jnp.maximum(x, y) for x, y in zip(a, b)], k0,
                     _cols(_tree(jnp.maximum, _rows(s))))
                if use_vpu and k0 == 0:
                    wrap_q((qr1, qr0)[j % 2], jnp.minimum(4 * i1 + j + 1, NC * H - 1))
                for tile in vpu[k0 // KC]:
                    assert VPU_STEPS[tile[0]] <= k0 // KC
                    vpu_scores(j, *tile)
                if k0 + KC == S:
                    m = jnp.max(jnp.concatenate(st["m"], axis=1), axis=0, keepdims=True)
                    new_ms.append(jnp.broadcast_to(m, (8, TC)))
            if i2 is not None:
                rows = pl.ds(pl.multiple_of((i2 & 7) * 128 + j * DH, DH), DH)
                ps = [jnp.exp2(r - ms[j]) for r in _rows(s_old)]
                fold("l", jnp.add, k0, _tree(jnp.add, ps))
                p = jnp.concatenate(ps, axis=0).astype(BF16)
                fold("o", jnp.add, k0,
                     jnp.dot(vt[kc, rows, t0:t0 + KC], p, preferred_element_type=F32))
                if k0 + KC == S:
                    act[i2 >> 3, rows, :] = st["o"] * (
                        1.0 / jnp.sum(st["l"], axis=0, keepdims=True))

        return [lambda j=j, k0=k0: job(j, k0) for j in range(4) for k0 in range(0, S, KC)]

    def layer_b(waits=(), side=()):
        def attn(i1, i2, ms):
            new_ms = []
            _run(attn_jobs(i1, i2, ms, new_ms))
            return tuple(new_ms)

        n = NC * NG
        a_out(0)
        _run(stats_jobs(0))
        lax.fori_loop(0, NC - 1, lambda c, _: b_chunk(c), None)
        _run(waits)
        skew_keys()
        wrap_q(qr0, 4 + zero())
        b_chunk(NC - 1, side)
        ms = attn(zero(), None, None)
        ms = lax.fori_loop(0, n - 1, lambda i, ms: attn(i + 1, i, ms), ms)
        return attn_jobs(None, n - 1, ms, None)

    def first_layer():
        stage = ((qt, 0), (qt, 2), (vt, 0), (vt, 2), (vt, 0), (qt, 0))

        def x_copy(c):
            return pltpu.make_async_copy(
                x_hbm.at[0, pl.ds(c * TC, TC), :], io_buf.at[c], sem_x.at[c])

        def w_copy(m, u):
            src, col = ((wa_hbm, D), (wa_hbm, 2 * D), (wa_hbm, 0),
                        (wb_hbm, 0), (wb_hbm, D), (wb_hbm, 2 * D))[m]
            buf, slot = stage[m]
            return pltpu.make_async_copy(src.at[:, pl.ds(col + u * TC, TC)],
                                         buf.at[slot + u], sem_w.at[2 * m + u])

        def wob_copy(u):
            return pltpu.make_async_copy(
                wob_hbm.at[pl.ds(u * TC, TC), :], io_buf.at[u], sem_w.at[12 + u])

        def woa_copy():
            return pltpu.make_async_copy(woa_hbm, woa, sem_w.at[14])

        def x_jobs(c):
            z = zero()

            def job(r):
                xt[c, r:r + 128, :] = io_buf[c, :, r:r + 128].astype(F32).T
                return [xt[c + z, r:r + 8, :128]]
            return [lambda r=r: job(r) for r in range(0, D, 128)] + stats_jobs(c)

        def transpose_jobs(load):
            z = zero()

            def job(r, l):
                wt[r // DB, r % DB:r % DB + 128, l:l + TC] = load(r, l).T
                return [wt[r // DB + z, r % DB:r % DB + 8, l:l + 128].astype(F32)]
            return [lambda r=r, l=l: job(r, l)
                    for r in range(0, D, 128) for l in range(0, D, TC)]

        def staged(buf, slot):
            return lambda r, l: buf[slot + r // TC, l:l + TC, r % TC:r % TC + 128]

        def w_jobs(w, fine=False):
            z = zero()
            return expand_jobs(w, lambda i, j, r: wt[
                i + z, r:r + 8, j * DB:(j + 1) * DB].astype(F32), fine)

        w_copy(0, 0).start()
        a_reset()
        w_copy(0, 1).start()
        jobs = transpose_jobs(staged(*stage[0]))
        w_copy(0, 0).wait()
        x_copy(0).start()
        _run(jobs[:8])
        w_copy(0, 1).wait()
        w_copy(1, 0).start()
        _run(jobs[8:] + w_jobs(wak))
        x_copy(0).wait()
        w_copy(1, 1).start()
        w_copy(2, 0).start()
        w_copy(2, 1).start()
        x_copy(1).start()
        _run(x_jobs(0))

        def transfers(i):
            if i == 0:
                w_copy(1, 0).wait()
                w_copy(1, 1).wait()
                _run(transpose_jobs(staged(*stage[1])) + w_jobs(wav))
            for u in range(2):
                w_copy(2 + i, u).wait()
            x_copy(i + 1).wait()
            for u in range(2):
                w_copy(3 + i, u).start()
            (x_copy(i + 2) if i < 2 else woa_copy()).start()
            if i:
                wob_copy(i - 1).start()

        def body(c, _):
            terms = ln_terms(c)
            pk = a_k(terms)
            for i in range(NC - 1):
                pl.when(c == i)(lambda i=i: transfers(i))
            v = a_v(terms, (0, 12, transpose_jobs(staged(vt, 2 * (c & 1)))),
                    (12, NP - 3, w_jobs(wqk.at[c])))
            a_q(c, terms, (0, NP - 4, x_jobs(c + 1)))
            _run(kv_jobs(pk, v))

        lax.fori_loop(0, NC - 1, body, None)
        woa_copy().wait()
        w_copy(5, 0).wait()
        w_copy(5, 1).wait()
        a_last_chunk([(20, NP - 4, transpose_jobs(staged(*stage[5])))],
                     [(0, NP - 4, w_jobs(wbv, True))])
        return ([wob_copy(0).wait, wob_copy(1).wait],
                ((0, NP - 4, transpose_jobs(lambda r, l: io_buf[l // TC, :, r:r + 128])),
                 (0, NP - 4, w_jobs(wbo, True))))

    def third_layer(attn_rest):
        def residual(c, *side):
            for r, t, b in b_out(c, *side):
                xt[c, r, t] += b

        def body(c, _):
            terms = ln_terms(c)
            v = a_v(terms)
            pk = a_k(terms)
            residual(c + 1)
            a_q(c, terms, (2, NP - 16, stats_jobs(c + 1)))
            _run(kv_jobs(pk, v))

        n = len(attn_rest) * 7 // 8
        a_reset()
        residual(0, (0, NP, attn_rest[:n]))
        _run(attn_rest[n:] + stats_jobs(0))
        lax.fori_loop(0, NC - 1, body, None)
        a_last_chunk()

    def output(attn_rest):
        def o_copy(c, q):
            r, t = _DONE[q][0] * D // 2, _DONE[q][1] * TC // 2
            return pltpu.make_async_copy(
                io_buf.at[c, pl.ds(t, TC // 2), pl.ds(r, D // 2)],
                out_hbm.at[0, pl.ds(c * TC + t, TC // 2), pl.ds(r, D // 2)],
                sem_o.at[4 * c + q])

        def emit(c, *side):
            for i, (r, t, b) in enumerate(b_out(c, *side)):
                io_buf[c, t, r] = (xt[c, r, t] + b).astype(BF16).T
                if i % 4 == 3:
                    o_copy(c, i // 4).start()

        emit(0, (0, NP, attn_rest))
        lax.fori_loop(1, NC, lambda c, _: emit(c), None)
        for c in range(NC):
            for q in range(4):
                o_copy(c, q).wait()

    third_layer(layer_b(*first_layer()))
    output(layer_b())


@jax.jit
def pallas_interleave_layers__linear_attn_block__mha_block__prompt_kernel(
    A_x: jax.Array,
    A_wqkv: jax.Array,
    A_wo: jax.Array,
    B_x: jax.Array,
    B_wqkv: jax.Array,
    B_wo: jax.Array,
):
    del B_x
    any_spec = pl.BlockSpec(memory_space=pl.ANY)
    return pl.pallas_call(
        _kernel,
        out_shape=jax.ShapeDtypeStruct((1, S, D), BF16),
        in_specs=[any_spec] * 5,
        out_specs=any_spec,
        scratch_shapes=[
            pltpu.VMEM((NC, TC, D), BF16),
            pltpu.VMEM((D, D), BF16),
            *[pltpu.VMEM((NP, DB, DB), BF16)] * 5,
            pltpu.VMEM((3, NP, DB, DB), BF16),
            pltpu.VMEM((NB, DB, D), BF16),
            pltpu.VMEM((NC, D, TC), F32),
            pltpu.VMEM((2, 8, TC), F32),
            pltpu.VMEM((NC, D, TC), F32),
            pltpu.VMEM((NG, 128, 128), F32),
            pltpu.VMEM((D, 128), F32),
            pltpu.VMEM((4, S, TC), F32),
            pltpu.VMEM((NC, D, TC), BF16),
            pltpu.VMEM((NG, NC, TC, 128), BF16),
            pltpu.VMEM((NC, D, TC), BF16),
            pltpu.VMEM((NG, 16 * len(VPU_STEPS), 128), F32),
            *[pltpu.VMEM((TC // 128, DH + 8, 128), F32)] * 2,
            pltpu.SMEM((2,), I32),
            pltpu.SemaphoreType.DMA((NC,)),
            pltpu.SemaphoreType.DMA((15,)),
            pltpu.SemaphoreType.DMA((4 * NC,)),
        ],
        compiler_params=pltpu.CompilerParams(vmem_limit_bytes=124 * 1024 * 1024),
        name="interleave_kernel",
    )(A_x, A_wqkv, A_wo, B_wqkv, B_wo)
```

```python
import functools
import math

import jax
import jax.numpy as jnp
from jax import lax
import jax.experimental.pallas as pl
import jax.experimental.pallas.tpu as pltpu

S, D, H, DH = 2048, 1024, 32, 32
TC = 512
NC = S // TC
NG = D // 128
KC = 128
VPU_STEPS = (0, 4, 8, 11)
NB, NP = 4, 49
DB, TB = D // NB, TC // NB
F32, BF16, I32 = jnp.float32, jnp.bfloat16, jnp.int32
QSCALE = DH ** -0.5 * math.log2(math.e)

_TN = (((0,), (0,)), ((), ()))
_NT = (((1,), (1,)), ((), ()))


def _tree(op, xs):
    xs = list(xs)
    while len(xs) > 1:
        xs = [op(xs[i], xs[i + 1]) if i + 1 < len(xs) else xs[i]
              for i in range(0, len(xs), 2)]
    return xs[0]


def _tiles(x):
    return x.reshape(x.shape[0] // 8, 8, x.shape[1])


def _pairwise_sum(x):
    while x.shape[0] > 2:
        x = jnp.sum(x.reshape(x.shape[0] // 2, 2, *x.shape[1:]), axis=1)
    return jnp.sum(x, axis=0)


def _cols(x):
    return [x[:, i:i + 128] for i in range(0, x.shape[1], 128)]


def _sublane_sum(x):
    return jnp.broadcast_to(jnp.sum(x, axis=0, keepdims=True), x.shape)


def _bcast_rows(v, n):
    return jnp.concatenate([v] * (n // 8), axis=0)


def _phi(t):
    return jnp.where(t > 0, t + 1.0, jnp.exp(t)) + 1e-6


def _add(a, b):
    return [[x + y for x, y in zip(r, s)] for r, s in zip(a, b)]


def _sub(a, b):
    return [[x - y for x, y in zip(r, s)] for r, s in zip(a, b)]


_LHS = (((1, 0), _add, (1, 1)), ((0, 0), _add, (1, 1)), ((1, 1),), ((0, 0),),
        ((0, 0), _add, (0, 1)), ((1, 0), _sub, (0, 0)), ((0, 1), _sub, (1, 1)))
_RHS = (((0, 0),), ((0, 0), _sub, (1, 1)), ((1, 0), _sub, (0, 0)), ((0, 1), _sub, (1, 1)),
        ((1, 1),), ((0, 0), _sub, (0, 1)), ((1, 0), _sub, (1, 1)))
_DONE = ((1, 0), (0, 1), (1, 1), (0, 0))


def _operand(term, quad):
    return term[1](quad(*term[0]), quad(*term[2])) if len(term) > 1 else quad(*term[0])


def _terms(table, x):
    if len(x) == 1:
        yield x[0][0]
        return
    n = len(x) // 2
    for term in table:
        yield from _terms(table, _operand(
            term, lambda i, j: [r[j * n:(j + 1) * n] for r in x[i * n:(i + 1) * n]]))


def _combine(products, n=NB):
    if n == 1:
        return [[next(products)]]
    m2 = _combine(products, n // 2)
    m1 = _combine(products, n // 2)
    c22 = _sub(m2, m1)
    m4 = _combine(products, n // 2)
    c21, c11 = _add(m2, m4), _add(m1, m4)
    m3 = _combine(products, n // 2)
    c22 = _add(c22, m3)
    m5 = _combine(products, n // 2)
    c12, c11 = _add(m3, m5), _add(c11, m5)
    c22 = _sub(c22, _combine(products, n // 2))
    c11 = _add(c11, _combine(products, n // 2))
    return [r + s for r, s in zip(c11, c12)] + [r + s for r, s in zip(c21, c22)]


def _blk(i, j):
    return slice(i * DB, (i + 1) * DB), slice(j * TB, (j + 1) * TB)


def _rhs_terms(block):
    grid = [[block(*_blk(i, j)) for j in range(NB)] for i in range(NB)]
    return [t.astype(BF16) for t in _terms(_RHS, grid)]


def _each(blocks):
    idx = [(2 * i + a, 2 * j + b) for i, j in _DONE for a, b in _DONE]
    return [(*_blk(i, j), blocks[i][j]) for i, j in idx]


def _run(jobs):
    for job in jobs:
        job()


def _spread(n, parts, odd=0):
    slots = [[] for _ in range(n)]
    for first, last, jobs in parts:
        for i, job in enumerate(jobs):
            p = first + i * (last - first) // len(jobs)
            slots[min(p | odd, n - 1)].append(job)
    return slots


def _after(x, tokens, zero):
    never = jnp.full((8, 128), zero, I32) != 0
    cols = _cols(pltpu.bitcast(x, I32))
    for tok in tokens:
        cols[-1] = jnp.where(never, pltpu.bitcast(tok, I32), cols[-1])
    return pltpu.bitcast(jnp.concatenate(cols, axis=1), BF16)


def _kernel(x_hbm, wa_hbm, woa_hbm, wb_hbm, wob_hbm, out_hbm,
            io_buf, woa, wak, wav, wao, wbv, wbo, wqk, wt,
            xt, stat, act, kvt, zacc, s_buf,
            qt, kk, vt, ks, qr0, qr1, zero_ref, sem_x, sem_w, sem_o):
    waq, wbq, wbk = wqk.at[0], wqk.at[1], wqk.at[2]

    def clear(i, _):
        zero_ref[i] = 0

    lax.fori_loop(0, 2, clear, None)
    uses = iter(range(1, 1000))

    def zero():
        return zero_ref[0] * next(uses)

    def project(w, terms, *side):
        z = zero()
        due = {}

        def products():
            for p, jobs in enumerate(_spread(NP, side, odd=1)):
                if due.get(p):
                    lhs = jnp.concatenate(
                        [w[p + z, :DB - 16, :], _after(w[p + z, DB - 16:, :], due[p], z)],
                        axis=0)
                else:
                    lhs = w[p + z]
                result = jnp.dot(lhs, terms[p], preferred_element_type=F32)
                due[p + 3] = [tok for job in jobs for tok in job() or ()]
                yield result
        return _combine(products())

    def expand_jobs(w, load, fine):
        z = zero()

        def job(r, qs):
            quad = functools.cache(lambda i, j: [
                [load(2 * i + a, 2 * j + b, r) for b in range(2)] for a in range(2)])
            for q in qs:
                for p, t in enumerate(_terms(_LHS, _operand(_LHS[q], quad))):
                    w[7 * q + p, r, :] = t.astype(BF16)
            return [w[7 * qs[-1] + z, r.stop - 8:r.stop, :128].astype(F32)]

        if fine:
            return [lambda r=r, q=q: job(slice(r, r + 16), [q])
                    for q in range(7) for r in range(0, DB, 16)]
        return [lambda r=r: job(slice(r, r + 8), range(7)) for r in range(0, DB, 8)]

    def stats_jobs(c, step=64):
        acc = {}
        z = zero()

        def mean(r):
            x = xt[c + z, r:r + step, :]
            t = jnp.sum(_tiles(jnp.concatenate([acc[0], x], axis=0) if r else x), axis=0)
            acc[0] = _sublane_sum(t) * (1.0 / D) if r + step == D else t
            return _cols(acc[0])

        def variance(r):
            x = xt[c - z, r:r + step, :] - _bcast_rows(acc[0], step)
            x = x * x
            t = jnp.sum(_tiles(jnp.concatenate([acc[1], x], axis=0) if r else x), axis=0)
            acc[1] = t
            if r + step == D:
                stat[0] = acc[0]
                stat[1] = lax.rsqrt(_sublane_sum(t) * (1.0 / D) + 1e-5)
            return _cols(t)

        return [lambda f=f, r=r: f(r) for f in (mean, variance) for r in range(0, D, step)]

    def ln_terms(c):
        mean, rstd = stat[0], stat[1]
        c = c + zero()
        return _rhs_terms(lambda r, t: (
            (xt[c, r, t] - _bcast_rows(mean[:, t], DB)) * _bcast_rows(rstd[:, t], DB)))

    def a_reset():
        kvt[...] = jnp.zeros_like(kvt)
        zacc[...] = jnp.zeros_like(zacc)

    def groups(blocks):
        return [jnp.concatenate([b[r:r + 128] for b in row], axis=1).astype(BF16)
                for row in blocks for r in range(0, DB, 128)]

    def a_k(terms, *side):
        pk = [[_phi(b) for b in row] for row in project(wak, terms, *side)]
        for i, row in enumerate(pk):
            zacc[i * DB:(i + 1) * DB, :] += _tree(jnp.add, row)
        return groups(pk)

    def a_v(terms, *side):
        return groups(project(wav, terms, *side))

    def a_q(c, terms, *side):
        for r, t, b in _each(project(waq, terms, *side)):
            act[c, r, t] = _phi(b)

    def kv_jobs(pk, v):
        def job(g):
            kvt[g] += lax.dot_general(v[g], pk[g], _NT, preferred_element_type=F32)
        return [lambda g=g: job(g) for g in reversed(range(NG))]

    def mix_jobs():
        def job(g):
            r = lax.broadcasted_iota(I32, (128, 128), 0) // DH
            c = lax.broadcasted_iota(I32, (128, 128), 1) // DH
            gs = slice(g * 128, (g + 1) * 128)
            blk = jnp.where(r == c, kvt[g], 0.0).astype(BF16)
            s_buf[g // 2, :D, g % 2 * 128:(g % 2 + 1) * 128] = lax.dot_general(
                woa[gs, :], blk, _TN, preferred_element_type=F32)
            z = jnp.sum(zacc[gs, :], axis=1, keepdims=True)
            zacc[gs, :] = jnp.broadcast_to(z, (128, 128))
        return [lambda g=g: job(g) for g in reversed(range(NG))]

    def a_last_chunk(side_v=(), side_k=()):
        z = zero()
        terms = ln_terms(NC - 1)
        v = a_v(terms, *side_v)
        pk = a_k(terms, *side_k)
        a_q(NC - 1, terms, (5, 6, kv_jobs(pk, v) + mix_jobs()),
            (16, NP - 1, expand_jobs(
                wao, lambda i, j, r: s_buf[j + z, i * DB + r.start:i * DB + r.stop, :DB],
                False)))

    def a_out(c):
        c = c + zero()

        def normalised(r, t):
            p = act[c, r, t].reshape(DB // DH, DH, TB)
            den = jnp.sum(p * zacc[r, :].reshape(p.shape), axis=1, keepdims=True) + 1e-6
            return (p * (1.0 / den)).reshape(DB, TB)

        for r, t, b in _each(project(wao, _rhs_terms(normalised))):
            xt[c, r, t] += b

    def b_chunk(c, last=None):
        def store(ref, blocks, scale=None):
            for i, row in enumerate(blocks):
                for j in range(0, NB, 2):
                    b = jnp.concatenate(row[j:j + 2], axis=1)
                    ref[c, i * DB:(i + 1) * DB, j * TB:(j + 2) * TB] = (
                        b * scale if scale else b).astype(BF16)

        terms = ln_terms(c)
        for r, t, b in _each(project(wbk, terms)):
            for g in range(DB // 128):
                kk[r.start // 128 + g, c, t.start // 2:t.stop // 2, :] = pltpu.bitcast(
                    b[g * 128:(g + 1) * 128].astype(BF16).T, I32)
        if last is None:
            store(qt, project(wbq, terms), QSCALE)
            a_out(c + 1)
            store(vt, project(wbv, terms, (2, NP - 4, stats_jobs(c + 1))))
        else:
            store(qt, project(wbq, terms, *last[:1]), QSCALE)
            store(vt, project(wbv, terms, *last[1:]))

    def b_out(c, *side):
        return _each(project(wbo, _rhs_terms(lambda r, t: act[c, r, t]), *side))

    def keys(g, k0, n):
        return pltpu.bitcast(kk[g, k0 // TC, k0 % TC // 2:(k0 % TC + n) // 2, :], BF16)

    def skew_keys():
        first = [(n + 1) * KC - 16 for n in VPU_STEPS]
        for g in range(NG):
            x = jnp.concatenate([keys(g, k, 16) for k in first], axis=0).astype(F32)
            row = lax.broadcasted_iota(I32, x.shape, 0)
            lane = lax.broadcasted_iota(I32, x.shape, 1) & (DH - 1)
            for b in (1, 2, 4):
                ahead = jnp.concatenate([x[:, b:], x[:, :b]], axis=1)
                wrapped = jnp.concatenate([x[:, b - DH:], x[:, :b - DH]], axis=1)
                x = jnp.where((row & b) == 0, x, jnp.where(lane < DH - b, ahead, wrapped))
            ks[g] = x

    def head_q(h):
        return qt[h >> 5, pl.ds(pl.multiple_of((h & 31) * DH, DH), DH), :]

    def wrap_q(ref, h):
        for u, q in enumerate(_cols(head_q(h).astype(F32))):
            ref[u] = jnp.concatenate([q, q[:8]], axis=0)

    def attn_jobs(i1, i2, ms, new_ms):
        st = {}
        use_vpu = i1 is not None and i2 is not None
        tiles = [(n, u, zero()) for n in range(len(VPU_STEPS))
                 for u in (0, 2)] if use_vpu else []
        vpu = _spread(S // KC, [(4, 17, tiles)])

        def fold(name, op, k0, val):
            st[name] = op(st[name], val) if k0 else val

        def vpu_scores(j, n, u, z):
            k = ks[(i1 & 7) + z, 16 * n:16 * n + 16, :].reshape(2, 1, 8, 128)
            for d in range(DH):
                t = k[..., j * DH + d:j * DH + d + 1] * (
                    (qr0, qr1)[j % 2][u:u + 2, pl.ds(z + d, 8), :])
                acc = acc + t if d else t
            row = (VPU_STEPS[n] + 1) * KC - 16
            for w in range(2):
                s_buf[j, row:row + 16, (u + w) * 128:(u + w + 1) * 128] = (
                    acc[:, w].reshape(16, 128))
                st["m"][u + w] = jnp.maximum(st["m"][u + w], jnp.max(acc[:, w], axis=0))

        def job(j, k0):
            kc, t0 = k0 // TC, k0 % TC
            if i2 is not None:
                s_old = s_buf[j, k0:k0 + KC, :]
            if i1 is not None:
                if k0 == 0:
                    q = head_q(4 * i1 + j)
                    st["q"] = jnp.concatenate(
                        [q if u == j else jnp.zeros_like(q) for u in range(4)], axis=0)
                nk = KC - 16 if use_vpu and k0 // KC in VPU_STEPS else KC
                s = jnp.dot(keys(i1 & 7, k0, nk), st["q"], preferred_element_type=F32)
                s_buf[j, k0:k0 + nk, :] = s
                fold("m", lambda a, b: [jnp.maximum(x, y) for x, y in zip(a, b)], k0,
                     _cols(jnp.max(_tiles(s), axis=0)))
                if use_vpu and k0 == 0:
                    wrap_q((qr1, qr0)[j % 2], jnp.minimum(4 * i1 + j + 1, NC * H - 1))
                for tile in vpu[k0 // KC]:
                    assert VPU_STEPS[tile[0]] <= k0 // KC
                    vpu_scores(j, *tile)
                if k0 + KC == S:
                    m = jnp.max(jnp.concatenate(st["m"], axis=1), axis=0, keepdims=True)
                    new_ms.append(jnp.broadcast_to(m, (8, TC)))
            if i2 is not None:
                rows = pl.ds(pl.multiple_of((i2 & 7) * 128 + j * DH, DH), DH)
                p = jnp.exp2(s_old - _bcast_rows(ms[j], KC))
                fold("l", jnp.add, k0, _pairwise_sum(_tiles(p)))
                fold("o", jnp.add, k0, jnp.dot(vt[kc, rows, t0:t0 + KC], p.astype(BF16),
                                               preferred_element_type=F32))
                if k0 + KC == S:
                    act[i2 >> 3, rows, :] = st["o"] * (
                        1.0 / jnp.sum(st["l"], axis=0, keepdims=True))

        return [lambda j=j, k0=k0: job(j, k0) for j in range(4) for k0 in range(0, S, KC)]

    def layer_b(waits=(), side=()):
        def attn(i1, i2, ms):
            new_ms = []
            _run(attn_jobs(i1, i2, ms, new_ms))
            return tuple(new_ms)

        n = NC * NG

        @pl.when(zero() == 0)
        def _():
            a_out(0)
            _run(stats_jobs(0))

        lax.fori_loop(0, NC - 1, lambda c, _: b_chunk(c), None)
        _run(waits)
        skew_keys()
        wrap_q(qr0, 4 + zero())
        b_chunk(NC - 1, side)
        ms = attn(zero(), None, None)
        ms = lax.fori_loop(0, n - 1, lambda i, ms: attn(i + 1, i, ms), ms)
        return attn_jobs(None, n - 1, ms, None)

    def first_layer():
        stage = ((qt, 0), (qt, 2), (vt, 0), (vt, 2), (vt, 0), (qt, 0))

        def x_copy(c):
            return pltpu.make_async_copy(
                x_hbm.at[0, pl.ds(c * TC, TC), :], io_buf.at[c], sem_x.at[c])

        def w_copy(m, u):
            src, col = ((wa_hbm, D), (wa_hbm, 2 * D), (wa_hbm, 0),
                        (wb_hbm, 0), (wb_hbm, D), (wb_hbm, 2 * D))[m]
            buf, slot = stage[m]
            return pltpu.make_async_copy(src.at[:, pl.ds(col + u * TC, TC)],
                                         buf.at[slot + u], sem_w.at[2 * m + u])

        def wob_copy(u):
            return pltpu.make_async_copy(
                wob_hbm.at[pl.ds(u * TC, TC), :], io_buf.at[u], sem_w.at[12 + u])

        def woa_copy():
            return pltpu.make_async_copy(woa_hbm, woa, sem_w.at[14])

        def x_jobs(c):
            z = zero()

            def job(r):
                xt[c, r:r + 128, :] = io_buf[c, :, r:r + 128].astype(F32).T
                return [xt[c + z, r:r + 8, :128]]
            return [lambda r=r: job(r) for r in range(0, D, 128)] + stats_jobs(c)

        def transpose_jobs(load):
            z = zero()

            def job(r, l):
                wt[r // DB, r % DB:r % DB + 128, l:l + TC] = load(r, l).T
                return [wt[r // DB + z, r % DB:r % DB + 8, l:l + 128].astype(F32)]
            return [lambda r=r, l=l: job(r, l)
                    for r in range(0, D, 128) for l in range(0, D, TC)]

        def staged(buf, slot):
            return lambda r, l: buf[slot + r // TC, l:l + TC, r % TC:r % TC + 128]

        def w_jobs(w, fine=False):
            z = zero()
            return expand_jobs(w, lambda i, j, r: wt[
                i + z, r, j * DB:(j + 1) * DB].astype(F32), fine)

        def start():
            w_copy(0, 0).start()
            a_reset()
            w_copy(0, 1).start()
            jobs = transpose_jobs(staged(*stage[0]))
            w_copy(0, 0).wait()
            x_copy(0).start()
            _run(jobs[:8])
            w_copy(0, 1).wait()
            w_copy(1, 0).start()
            _run(jobs[8:] + w_jobs(wak))
            x_copy(0).wait()
            w_copy(1, 1).start()
            w_copy(2, 0).start()
            w_copy(2, 1).start()
            x_copy(1).start()
            _run(x_jobs(0))

        def transfers(i):
            if i == 0:
                w_copy(1, 0).wait()
                w_copy(1, 1).wait()
                _run(transpose_jobs(staged(*stage[1])) + w_jobs(wav))
            for u in range(2):
                w_copy(2 + i, u).wait()
            x_copy(i + 1).wait()
            for u in range(2):
                w_copy(3 + i, u).start()
            (x_copy(i + 2) if i < 2 else woa_copy()).start()
            if i:
                wob_copy(i - 1).start()

        def body(c, _):
            terms = ln_terms(c)
            pk = a_k(terms)
            for i in range(NC - 1):
                pl.when(c == i)(lambda i=i: transfers(i))
            v = a_v(terms, (0, 18, transpose_jobs(staged(vt, 2 * (c & 1)))),
                    (18, NP - 3, w_jobs(wqk.at[c])))
            jobs = x_jobs(c + 1)
            a_q(c, terms, (0, 6, jobs[:8]), (6, NP - 4, jobs[8:]))
            _run(kv_jobs(pk, v))

        start()
        lax.fori_loop(0, NC - 1, body, None)
        woa_copy().wait()
        w_copy(5, 0).wait()
        w_copy(5, 1).wait()
        a_last_chunk([(40, NP - 1, transpose_jobs(staged(*stage[5])))],
                     [(10, NP - 4, w_jobs(wbv, True))])
        return ([wob_copy(0).wait, wob_copy(1).wait],
                ((0, NP - 4, transpose_jobs(lambda r, l: io_buf[l // TC, :, r:r + 128])),
                 (0, NP - 4, w_jobs(wbo, True))))

    def third_layer(attn_rest):
        def residual(c, *side):
            for r, t, b in b_out(c, *side):
                xt[c, r, t] += b

        def body(c, _):
            terms = ln_terms(c)
            v = a_v(terms)
            pk = a_k(terms)
            residual(c + 1)
            a_q(c, terms, (2, NP - 16, stats_jobs(c + 1)))
            _run(kv_jobs(pk, v))

        a_reset()
        residual(0, (0, NP, attn_rest))
        _run(stats_jobs(0))
        lax.fori_loop(0, NC - 1, body, None)
        a_last_chunk()

    def output(attn_rest):
        def o_copy(c, q):
            r, t = _DONE[q][0] * D // 2, _DONE[q][1] * TC // 2
            return pltpu.make_async_copy(
                io_buf.at[c, pl.ds(t, TC // 2), pl.ds(r, D // 2)],
                out_hbm.at[0, pl.ds(c * TC + t, TC // 2), pl.ds(r, D // 2)],
                sem_o.at[4 * c + q])

        def emit(c, *side):
            for i, (r, t, b) in enumerate(b_out(c, *side)):
                io_buf[c, t, r] = (xt[c, r, t] + b).astype(BF16).T
                if i % 4 == 3:
                    o_copy(c, i // 4).start()

        emit(0, (0, NP, attn_rest))
        lax.fori_loop(1, NC, lambda c, _: emit(c), None)
        for c in range(NC):
            for q in range(4):
                o_copy(c, q).wait()

    third_layer(layer_b(*first_layer()))
    output(layer_b())


@jax.jit
def pallas_interleave_layers__linear_attn_block__mha_block__prompt_kernel(
    A_x: jax.Array,
    A_wqkv: jax.Array,
    A_wo: jax.Array,
    B_x: jax.Array,
    B_wqkv: jax.Array,
    B_wo: jax.Array,
):
    del B_x
    any_spec = pl.BlockSpec(memory_space=pl.ANY)
    return pl.pallas_call(
        _kernel,
        out_shape=jax.ShapeDtypeStruct((1, S, D), BF16),
        in_specs=[any_spec] * 5,
        out_specs=any_spec,
        scratch_shapes=[
            pltpu.VMEM((NC, TC, D), BF16),
            pltpu.VMEM((D, D), BF16),
            *[pltpu.VMEM((NP, DB, DB), BF16)] * 5,
            pltpu.VMEM((3, NP, DB, DB), BF16),
            pltpu.VMEM((NB, DB, D), BF16),
            pltpu.VMEM((NC, D, TC), F32),
            pltpu.VMEM((2, 8, TC), F32),
            pltpu.VMEM((NC, D, TC), F32),
            pltpu.VMEM((NG, 128, 128), F32),
            pltpu.VMEM((D, 128), F32),
            pltpu.VMEM((4, S, TC), F32),
            pltpu.VMEM((NC, D, TC), BF16),
            pltpu.VMEM((NG, NC, TC // 2, 128), I32),
            pltpu.VMEM((NC, D, TC), BF16),
            pltpu.VMEM((NG, 16 * len(VPU_STEPS), 128), F32),
            *[pltpu.VMEM((TC // 128, DH + 8, 128), F32)] * 2,
            pltpu.SMEM((2,), I32),
            pltpu.SemaphoreType.DMA((NC,)),
            pltpu.SemaphoreType.DMA((15,)),
            pltpu.SemaphoreType.DMA((4 * NC,)),
        ],
        compiler_params=pltpu.CompilerParams(vmem_limit_bytes=124 * 1024 * 1024),
        name="interleave_kernel",
    )(A_x, A_wqkv, A_wo, B_wqkv, B_wo)
```
